```python
import os as _os
_os.environ.setdefault("JAX_PLATFORMS", "cpu")
import jax
import jax.numpy as jnp

def _softmax(x, axis=-1):
    return jax.nn.softmax(x, axis=axis)
def _gelu(x):
    return jax.nn.gelu(x, approximate=True)
def _silu(x):
    return jax.nn.silu(x)
def _sigmoid(x):
    return jax.nn.sigmoid(x)
def _layernorm(x, axis=-1, eps=1e-5):
    m = jnp.mean(x, axis=axis, keepdims=True)
    v = jnp.var(x, axis=axis, keepdims=True)
    return (x - m) / jnp.sqrt(v + eps)
def _scatter_add(tgt, idx, src, axis=0):
    return tgt.at[idx].add(src)
def _segment_sum(src, seg, n):
    return jax.ops.segment_sum(src, seg, n)
class _Rng:
    def __init__(self, key):
        self._k = key
    def _next(self):
        self._k, sub = jax.random.split(self._k)
        return sub
    def normal(self, shape):
        return jax.random.normal(self._next(), shape, dtype=jnp.bfloat16)
    def randint(self, lo, hi, shape):
        return jax.random.randint(self._next(), shape, lo, hi, dtype=jnp.int32)
    def uniform(self, shape, lo=0.0, hi=1.0):
        return jax.random.uniform(self._next(), shape, jnp.bfloat16, lo, hi)
    def permutation(self, n):
        return jax.random.permutation(self._next(), n)


kernel_name = 'standalone__mha_softmax__sampling'

def setup_inputs():
    _rng = _Rng(jax.random.key(int.from_bytes(__import__("os").urandom(4), "little")))
    _w = (lambda a: (lambda t: t.astype(jnp.bfloat16) if jnp.issubdtype(t.dtype, jnp.floating) else t)(jnp.asarray(a)))
    B, H, Sq, Sk, D = 8, 32, 32, 2048, 128
    return {
        "q": _w((lambda *s: _rng.normal(s) * 0.4)(B, H, Sq, D)),
        "k": _w((lambda *s: _rng.normal(s) * 0.4)(B, H, Sk, D)),
        "v": _w((lambda *s: _rng.normal(s) * 0.05)(B, H, Sk, D)),
    }

def reference(q, k, v):
    scale = q.shape[-1] ** -0.5
    scores = jnp.einsum("bhqd,bhkd->bhqk", q, k) * scale
    p = _softmax(scores, axis=-1)
    return jnp.einsum("bhqk,bhkd->bhqd", p, v)
```

```python
import math

import jax
import jax.numpy as jnp
import jax.experimental.pallas as pl
import jax.experimental.pallas.tpu as pltpu

_CH = 128
_G = 4
_SP = 4
_A = 4
_NS = 3


def _attend(q, k, v, c):
    s = jax.lax.dot_general(
        q, k, (((1,), (1,)), ((), ())), preferred_element_type=jnp.float32)
    m = jnp.max(s, axis=-1, keepdims=True)
    p = jnp.exp2((s - m) * c)
    l = jnp.sum(p, axis=-1, keepdims=True)
    o = jnp.dot(p.astype(v.dtype), v, preferred_element_type=jnp.float32)
    return o / l


@jax.jit
def pallas_standalone__mha_softmax__sampling_kernel(
    q: jax.Array,
    k: jax.Array,
    v: jax.Array,
):
    b, nh, sq, d = q.shape
    sk = k.shape[2]
    n = b * nh
    hb = _G * _SP
    nu = n // _G
    nch = sk // _CH
    assert n % hb == 0 and sk % (_CH * _G) == 0
    c = (d ** -0.5) * math.log2(math.e)

    def kernel_function(q_hbm, k_hbm, v_hbm, o_hbm, qbuf, obuf, kbuf, vbuf, sem, osem):
        def q_copy(u):
            slot = u % _NS
            return pltpu.make_async_copy(
                q_hbm.at[u // _SP, :, u % _SP], qbuf.at[slot], sem.at[slot])

        def start(u, part):
            slot = u % _NS
            base = ((u // _SP) * hb + (u % _SP)) * sk
            per = nch // _G
            if part == 0:
                q_copy(u).start()
            for j in range(part * per, (part + 1) * per):
                for g in range(0, _G, 2):
                    for src, dst in ((k_hbm, kbuf), (v_hbm, vbuf)):
                        for p in range(2):
                            row = pl.multiple_of(base + (g + p) * _SP * sk + j * _CH, _CH)
                            pltpu.make_async_copy(
                                src.at[pl.ds(row, _CH)],
                                dst.at[slot, g + p, pl.ds(j * _CH, _CH)],
                                sem.at[slot]).start(priority=p)

        def wait(u):
            slot = u % _NS
            pltpu.make_async_copy(kbuf.at[slot], kbuf.at[slot], sem.at[slot]).wait()
            pltpu.make_async_copy(vbuf.at[slot], vbuf.at[slot], sem.at[slot]).wait()
            q_copy(u).wait()

        def compute(u, g):
            slot = u % _NS
            h = (u // _SP) * hb + (u % _SP) + g * _SP
            o = _attend(qbuf[slot, g], kbuf[slot, g], vbuf[slot, g], c)
            obuf[h] = o.astype(obuf.dtype)

        def o_start(h0, cnt, p):
            pltpu.make_async_copy(
                obuf.at[pl.ds(h0, cnt)], o_hbm.at[pl.ds(h0, cnt)], osem).start(priority=p)

        ahead = _G + _A - 1
        for i in range(ahead):
            start(i // _G, i % _G)

        def step(u, carry):
            for g in range(_G):
                start(u + (ahead + g) // _G, (ahead + g) % _G)
                if g == 0:
                    wait(u)
                compute(u, g)
            return carry

        nlast = (ahead + _G - 1) // _G
        jax.lax.fori_loop(0, nu - nlast, step, 0)
        for u in range(nu - nlast, nu):
            for g in range(_G):
                if u + (ahead + g) // _G < nu:
                    start(u + (ahead + g) // _G, (ahead + g) % _G)
                if g == 0:
                    wait(u)
                    if u == nu - 1:
                        half = (n - hb) // 2
                        o_start(0, half, 0)
                        o_start(half, half, 1)
                compute(u, g)
        o_start(n - hb, hb // 2, 0)
        o_start(n - hb // 2, hb // 2, 1)
        pltpu.make_async_copy(obuf, obuf, osem).wait()

    out = pl.pallas_call(
        kernel_function,
        in_specs=[pl.BlockSpec(memory_space=pl.ANY)] * 3,
        out_specs=pl.BlockSpec(memory_space=pl.ANY),
        out_shape=jax.ShapeDtypeStruct((n, sq, d), q.dtype),
        scratch_shapes=[
            pltpu.VMEM((_NS, _G, sq, d), q.dtype),
            pltpu.VMEM((n, sq, d), q.dtype),
            pltpu.VMEM((_NS, _G, sk, d), k.dtype),
            pltpu.VMEM((_NS, _G, sk, d), v.dtype),
            pltpu.SemaphoreType.DMA((_NS,)),
            pltpu.SemaphoreType.DMA,
        ],
        compiler_params=pltpu.CompilerParams(vmem_limit_bytes=64 * 2**20),
    )(q.reshape(n // hb, _G, _SP, sq, d), k.reshape(n * sk, d), v.reshape(n * sk, d))
    return out.reshape(b, nh, sq, d)
```

```python
import math

import jax
import jax.numpy as jnp
import jax.experimental.pallas as pl
import jax.experimental.pallas.tpu as pltpu

_DMA_ROWS = 128
_GROUP = 4
_LAST_GROUP = 2
_STRIDE = 16
_AHEAD = 4
_SLOTS = 16
_LATE = 3
_OUT_STREAMS = 8


def _attend(q, k, v, c):
    s = jax.lax.dot_general(
        q, k, (((1,), (1,)), ((), ())), preferred_element_type=jnp.float32)
    m = jnp.max(s, axis=-1, keepdims=True)
    p = jnp.exp2((s - m) * c)
    l = jnp.sum(p, axis=-1, keepdims=True)
    o = jnp.dot(p.astype(v.dtype), v, preferred_element_type=jnp.float32)
    return o / l


@jax.jit
def pallas_standalone__mha_softmax__sampling_kernel(
    q: jax.Array,
    k: jax.Array,
    v: jax.Array,
):
    b, nh, sq, d = q.shape
    sk = k.shape[2]
    n = b * nh
    chunks = sk // _DMA_ROWS
    qh = _DMA_ROWS // sq
    ahead = _GROUP - 1 + _AHEAD
    assert n % (_GROUP * _STRIDE) == 0 and n % (qh * _OUT_STREAMS) == 0
    assert sk % (_DMA_ROWS * _GROUP) == 0 and _DMA_ROWS % sq == 0
    assert _STRIDE % qh == 0 and _GROUP % _LAST_GROUP == 0
    assert _SLOTS % _GROUP == 0 and ahead + _GROUP <= _SLOTS
    c = (d ** -0.5) * math.log2(math.e)

    def head_of(i):
        span = _GROUP * _STRIDE
        return (i // span) * span + (i % _GROUP) * _STRIDE + (i // _GROUP) % _STRIDE

    late = sorted(head_of(i) for i in range(n - _LATE, n))
    per_stream = n // qh // _OUT_STREAMS
    burst = []
    for j in range(per_stream):
        for s in range(_OUT_STREAMS):
            lo = (s * per_stream + j) * qh
            end = lo + qh
            for h in [x for x in late if lo <= x < end] + [end]:
                if h > lo:
                    burst.append((lo, h - lo))
                lo = h + 1

    def kernel_function(q_hbm, k_hbm, v_hbm, o_hbm,
                        q_buf, o_buf, kv_buf, kv_sem, q_sem, o_sem):
        def loads_q(i):
            return ((i // _GROUP) % _STRIDE) % qh == 0

        def q_copy(i):
            h = pl.multiple_of(head_of(i), qh)
            return pltpu.make_async_copy(
                q_hbm.at[pl.ds(h, qh)], q_buf.at[pl.ds(h, qh)], q_sem.at[i % _SLOTS])

        def stream_kv(t, group):
            first = (t // group) * group
            head0, slot0 = head_of(first), first % _SLOTS
            per = chunks // group
            for j in range(per):
                row = pl.multiple_of(
                    (chunks - 1 - ((t % group) * per + j)) * _DMA_ROWS, _DMA_ROWS)
                for a, src in enumerate((k_hbm, v_hbm)):
                    for w in range(group):
                        pltpu.make_async_copy(
                            src.at[head0 + w * _STRIDE, pl.ds(row, _DMA_ROWS)],
                            kv_buf.at[slot0 + w, a, pl.ds(row, _DMA_ROWS)],
                            kv_sem.at[slot0 + w],
                        ).start(priority=w % 2)

        def prefetch(t):
            @pl.when(jnp.logical_and(t < n, loads_q(t)))
            def _():
                q_copy(t).start()

            @pl.when(t < n - _GROUP)
            def _():
                stream_kv(t, _GROUP)

            @pl.when(jnp.logical_and(t >= n - _GROUP, t < n))
            def _():
                stream_kv(t, _LAST_GROUP)

        def write_out(head, count, priority):
            pltpu.make_async_copy(
                o_buf.at[pl.ds(head, count)], o_hbm.at[pl.ds(head, count)], o_sem,
            ).start(priority=priority)

        def prologue(t, carry):
            prefetch(t)
            return carry

        def step(i, carry):
            prefetch(i + ahead)

            @pl.when(i == n - _LATE)
            def _():
                for idx, (head, count) in enumerate(burst):
                    write_out(head, count, idx % 2)

            slot = i % _SLOTS
            pltpu.make_async_copy(kv_buf.at[slot], kv_buf.at[slot], kv_sem.at[slot]).wait()

            @pl.when(loads_q(i))
            def _():
                q_copy(i).wait()

            head = head_of(i)
            o = _attend(q_buf[head], kv_buf[slot, 0], kv_buf[slot, 1], c)
            o_buf[head] = o.astype(o_buf.dtype)

            @pl.when(i >= n - _LATE)
            def _():
                write_out(head, 1, 1)

            return carry

        jax.lax.fori_loop(0, ahead, prologue, 0)
        jax.lax.fori_loop(0, n, step, 0)
        pltpu.make_async_copy(o_buf, o_hbm, o_sem).wait()

    out = pl.pallas_call(
        kernel_function,
        in_specs=[pl.BlockSpec(memory_space=pl.ANY)] * 3,
        out_specs=pl.BlockSpec(memory_space=pl.ANY),
        out_shape=jax.ShapeDtypeStruct((n, sq, d), q.dtype),
        scratch_shapes=[
            pltpu.VMEM((n, sq, d), q.dtype),
            pltpu.VMEM((n, sq, d), q.dtype),
            pltpu.VMEM((_SLOTS, 2, sk, d), k.dtype),
            pltpu.SemaphoreType.DMA((_SLOTS,)),
            pltpu.SemaphoreType.DMA((_SLOTS,)),
            pltpu.SemaphoreType.DMA,
        ],
        compiler_params=pltpu.CompilerParams(vmem_limit_bytes=64 * 2**20),
    )(q.reshape(n, sq, d), k.reshape(n, sk, d), v.reshape(n, sk, d))
    return out.reshape(b, nh, sq, d)
```

```python
import math

import jax
import jax.numpy as jnp
import jax.experimental.pallas as pl
import jax.experimental.pallas.tpu as pltpu

_DMA_ROWS = 128
_GROUP = 4
_LAST_GROUP = 2
_STRIDE = 16
_AHEAD = 4
_SLOTS = 16
_LATE = 3
_IO_STREAMS = 8


def _attend(q, k, v, c):
    s = jax.lax.dot_general(
        q, k, (((1,), (1,)), ((), ())), preferred_element_type=jnp.float32)
    m = jnp.max(s, axis=-1, keepdims=True)
    p = jnp.exp2((s - m) * c)
    l = jnp.sum(p, axis=-1, keepdims=True)
    o = jnp.dot(p.astype(v.dtype), v, preferred_element_type=jnp.float32)
    return o / l


@jax.jit
def pallas_standalone__mha_softmax__sampling_kernel(
    q: jax.Array,
    k: jax.Array,
    v: jax.Array,
):
    b, nh, sq, d = q.shape
    sk = k.shape[2]
    n = b * nh
    chunks = sk // _DMA_ROWS
    qh = _DMA_ROWS // sq
    ahead = _GROUP - 1 + _AHEAD
    assert n % (_GROUP * _STRIDE) == 0 and n % (qh * _IO_STREAMS) == 0
    assert sk % (_DMA_ROWS * _GROUP) == 0 and _DMA_ROWS % sq == 0
    assert _GROUP % _LAST_GROUP == 0 and ahead <= n - _GROUP
    assert _SLOTS % _GROUP == 0 and ahead + _GROUP <= _SLOTS
    c = (d ** -0.5) * math.log2(math.e)

    def head_of(i):
        span = _GROUP * _STRIDE
        return ((i // span) * span + (i % _GROUP) * _STRIDE
                + _STRIDE - 1 - (i // _GROUP) % _STRIDE)

    per_stream = n // qh // _IO_STREAMS
    io_blocks = [(s * per_stream + j) * qh
                 for j in range(per_stream) for s in range(_IO_STREAMS)]
    late = sorted(head_of(i) for i in range(n - _LATE, n))
    burst = []
    for lo in io_blocks:
        end = lo + qh
        for h in [x for x in late if lo <= x < end] + [end]:
            if h > lo:
                burst.append((lo, h - lo))
            lo = h + 1
    full = n - _GROUP

    def kernel_function(q_hbm, k_hbm, v_hbm, o_hbm,
                        q_buf, o_buf, kv_buf, kv_sem, io_sem):
        def group_sem(first, group):
            if group == _GROUP:
                index = first // _GROUP
            else:
                index = full // _GROUP + (first - full) // group
            return kv_sem.at[index % (_SLOTS // _GROUP)]

        def stream_kv(t, group):
            first = (t // group) * group
            head0, slot0, sem = head_of(first), first % _SLOTS, group_sem(first, group)
            per = chunks // group
            for j in range(per):
                row = pl.multiple_of(
                    (chunks - 1 - ((t % group) * per + j)) * _DMA_ROWS, _DMA_ROWS)
                for a, src in enumerate((k_hbm, v_hbm)):
                    for w in range(group):
                        pltpu.make_async_copy(
                            src.at[head0 + w * _STRIDE, pl.ds(row, _DMA_ROWS)],
                            kv_buf.at[slot0 + w, a, pl.ds(row, _DMA_ROWS)],
                            sem,
                        ).start(priority=w % 2)

        def wait_kv(first, group):
            slots = kv_buf.at[pl.ds(first % _SLOTS, group)]
            pltpu.make_async_copy(slots, slots, group_sem(first, group)).wait()

        def write_out(head, count, priority):
            pltpu.make_async_copy(
                o_buf.at[pl.ds(head, count)], o_hbm.at[pl.ds(head, count)], io_sem,
            ).start(priority=priority)

        def prologue(t, carry):
            stream_kv(t, _GROUP)
            return carry

        def step(i, carry):
            t = i + ahead

            @pl.when(t < full)
            def _():
                stream_kv(t, _GROUP)

            @pl.when(jnp.logical_and(t >= full, t < n))
            def _():
                stream_kv(t, _LAST_GROUP)

            @pl.when(i == n - _LATE)
            def _():
                for idx, (head, count) in enumerate(burst):
                    write_out(head, count, idx % 2)

            @pl.when(jnp.logical_and(i < full, i % _GROUP == 0))
            def _():
                wait_kv(i, _GROUP)

            @pl.when(jnp.logical_and(i >= full, i % _LAST_GROUP == 0))
            def _():
                wait_kv(i, _LAST_GROUP)

            head, slot = head_of(i), i % _SLOTS
            o = _attend(q_buf[head], kv_buf[slot, 0], kv_buf[slot, 1], c)
            o_buf[head] = o.astype(o_buf.dtype)

            @pl.when(i >= n - _LATE)
            def _():
                write_out(head, 1, 1)

            return carry

        for idx, head in enumerate(io_blocks):
            pltpu.make_async_copy(
                q_hbm.at[pl.ds(head, qh)], q_buf.at[pl.ds(head, qh)], io_sem,
            ).start(priority=idx % 2)
        jax.lax.fori_loop(0, ahead, prologue, 0)
        pltpu.make_async_copy(q_hbm, q_buf, io_sem).wait()
        jax.lax.fori_loop(0, n, step, 0)
        pltpu.make_async_copy(o_buf, o_hbm, io_sem).wait()

    out = pl.pallas_call(
        kernel_function,
        in_specs=[pl.BlockSpec(memory_space=pl.ANY)] * 3,
        out_specs=pl.BlockSpec(memory_space=pl.ANY),
        out_shape=jax.ShapeDtypeStruct((n, sq, d), q.dtype),
        scratch_shapes=[
            pltpu.VMEM((n, sq, d), q.dtype),
            pltpu.VMEM((n, sq, d), q.dtype),
            pltpu.VMEM((_SLOTS, 2, sk, d), k.dtype),
            pltpu.SemaphoreType.DMA((_SLOTS // _GROUP,)),
            pltpu.SemaphoreType.DMA,
        ],
        compiler_params=pltpu.CompilerParams(vmem_limit_bytes=64 * 2**20),
    )(q.reshape(n, sq, d), k.reshape(n, sk, d), v.reshape(n, sk, d))
    return out.reshape(b, nh, sq, d)
```

```python
import math

import jax
import jax.numpy as jnp
import jax.experimental.pallas as pl
import jax.experimental.pallas.tpu as pltpu

_DMA_ROWS = 128
_GROUP = 8
_TAIL = ((12, 4), (4, 2))
_STRIDE = 16
_AHEAD = 11
_TAIL_AHEAD = 8
_SLOTS = 32
_SEMS = 4
_LATE = 4
_IO_STREAMS = 8


def _attend(q, k, v, c):
    s = jax.lax.dot_general(
        q, k, (((1,), (1,)), ((), ())), preferred_element_type=jnp.float32)
    m = jnp.max(s, axis=-1, keepdims=True)
    p = jnp.exp2((s - m) * c)
    l = jnp.sum(p, axis=-1, keepdims=True)
    o = jnp.dot(p.astype(v.dtype), v, preferred_element_type=jnp.float32)
    return o / l


@jax.jit
def pallas_standalone__mha_softmax__sampling_kernel(
    q: jax.Array,
    k: jax.Array,
    v: jax.Array,
):
    b, nh, sq, d = q.shape
    sk = k.shape[2]
    n = b * nh
    chunks = sk // _DMA_ROWS
    qh = _DMA_ROWS // sq
    assert n % (_GROUP * _STRIDE) == 0 and n % (qh * _IO_STREAMS) == 0
    assert sk % (_DMA_ROWS * _GROUP) == 0 and _DMA_ROWS % sq == 0
    assert _SLOTS % _GROUP == 0 and _AHEAD + _GROUP <= _SLOTS
    c = (d ** -0.5) * math.log2(math.e)

    phases = []
    first = groups = 0
    for count, size in ((n - sum(x for x, _ in _TAIL), _GROUP),) + _TAIL:
        phases.append((first, first + count, size, groups))
        first, groups = first + count, groups + count // size

    def head_of(i):
        span = _GROUP * _STRIDE
        return (i // span) * span + (i % _GROUP) * _STRIDE + (i // _GROUP) % _STRIDE

    per_stream = n // qh // _IO_STREAMS
    io_blocks = [(s * per_stream + j) * qh
                 for j in range(per_stream) for s in range(_IO_STREAMS)]
    late = sorted(head_of(i) for i in range(n - _LATE, n))
    burst = []
    for lo in io_blocks:
        end = lo + qh
        for h in [x for x in late if lo <= x < end] + [end]:
            if h > lo:
                burst.append((lo, h - lo))
            lo = h + 1

    def kernel_function(q_hbm, k_hbm, v_hbm, o_hbm,
                        q_buf, o_buf, kv_buf, kv_sem, io_sem):
        def in_phase(i, phase):
            return jnp.logical_and(i >= phase[0], i < phase[1])

        def group_sem(i, phase):
            start, _, size, before = phase
            return kv_sem.at[(before + (i - start) // size) % _SEMS]

        def start_kv(t, phase):
            size = phase[2]
            lead = (t // size) * size
            head0, slot0, sem = head_of(lead), lead % _SLOTS, group_sem(t, phase)
            per = chunks // size
            for j in range(per):
                row = pl.multiple_of(((t % size) * per + j) * _DMA_ROWS, _DMA_ROWS)
                for a, src in enumerate((k_hbm, v_hbm)):
                    for w in range(size):
                        pltpu.make_async_copy(
                            src.at[head0 + w * _STRIDE, pl.ds(row, _DMA_ROWS)],
                            kv_buf.at[slot0 + w, a, pl.ds(row, _DMA_ROWS)],
                            sem,
                        ).start(priority=w % 2)

        def wait_kv(i, phase):
            slots = kv_buf.at[pl.ds(i % _SLOTS, phase[2])]
            pltpu.make_async_copy(slots, slots, group_sem(i, phase)).wait()

        def start_out(head, count, priority):
            pltpu.make_async_copy(
                o_buf.at[pl.ds(head, count)], o_hbm.at[pl.ds(head, count)], io_sem,
            ).start(priority=priority)

        def prologue(t, carry):
            start_kv(t, phases[0])
            return carry

        def step(i, t):
            ahead = jnp.where(i <= phases[0][1] - _GROUP, _AHEAD, _TAIL_AHEAD)
            due = t <= i + ahead
            for phase in phases:
                @pl.when(jnp.logical_and(due, in_phase(t, phase)))
                def _():
                    start_kv(t, phase)

            @pl.when(i == n - _LATE)
            def _():
                for idx, (head, count) in enumerate(burst):
                    start_out(head, count, idx % 2)

            for phase in phases:
                @pl.when(jnp.logical_and(in_phase(i, phase), i % phase[2] == 0))
                def _():
                    wait_kv(i, phase)

            head, slot = head_of(i), i % _SLOTS
            o = _attend(q_buf[head], kv_buf[slot, 0], kv_buf[slot, 1], c)
            o_buf[head] = o.astype(o_buf.dtype)

            @pl.when(i >= n - _LATE)
            def _():
                start_out(head, 1, 1)

            return t + due.astype(jnp.int32)

        for idx, head in enumerate(io_blocks):
            pltpu.make_async_copy(
                q_hbm.at[pl.ds(head, qh)], q_buf.at[pl.ds(head, qh)], io_sem,
            ).start(priority=idx % 2)
        jax.lax.fori_loop(0, _AHEAD, prologue, 0)
        pltpu.make_async_copy(q_hbm, q_buf, io_sem).wait()
        jax.lax.fori_loop(0, n, step, _AHEAD)
        pltpu.make_async_copy(o_buf, o_hbm, io_sem).wait()

    out = pl.pallas_call(
        kernel_function,
        in_specs=[pl.BlockSpec(memory_space=pl.ANY)] * 3,
        out_specs=pl.BlockSpec(memory_space=pl.ANY),
        out_shape=jax.ShapeDtypeStruct((n, sq, d), q.dtype),
        scratch_shapes=[
            pltpu.VMEM((n, sq, d), q.dtype),
            pltpu.VMEM((n, sq, d), q.dtype),
            pltpu.VMEM((_SLOTS, 2, sk, d), k.dtype),
            pltpu.SemaphoreType.DMA((_SEMS,)),
            pltpu.SemaphoreType.DMA,
        ],
        compiler_params=pltpu.CompilerParams(vmem_limit_bytes=64 * 2**20),
    )(q.reshape(n, sq, d), k.reshape(n, sk, d), v.reshape(n, sk, d))
    return out.reshape(b, nh, sq, d)
```
